```python
import os as _os
_os.environ.setdefault("JAX_PLATFORMS", "cpu")
import jax
import jax.numpy as jnp

def _softmax(x, axis=-1):
    return jax.nn.softmax(x, axis=axis)
def _gelu(x):
    return jax.nn.gelu(x, approximate=True)
def _silu(x):
    return jax.nn.silu(x)
def _sigmoid(x):
    return jax.nn.sigmoid(x)
def _layernorm(x, axis=-1, eps=1e-5):
    m = jnp.mean(x, axis=axis, keepdims=True)
    v = jnp.var(x, axis=axis, keepdims=True)
    return (x - m) / jnp.sqrt(v + eps)
def _scatter_add(tgt, idx, src, axis=0):
    return tgt.at[idx].add(src)
def _segment_sum(src, seg, n):
    return jax.ops.segment_sum(src, seg, n)
class _Rng:
    def __init__(self, key):
        self._k = key
    def _next(self):
        self._k, sub = jax.random.split(self._k)
        return sub
    def normal(self, shape):
        return jax.random.normal(self._next(), shape, dtype=jnp.bfloat16)
    def randint(self, lo, hi, shape):
        return jax.random.randint(self._next(), shape, lo, hi, dtype=jnp.int32)
    def uniform(self, shape, lo=0.0, hi=1.0):
        return jax.random.uniform(self._next(), shape, jnp.bfloat16, lo, hi)
    def permutation(self, n):
        return jax.random.permutation(self._next(), n)


kernel_name = 'standalone__sliding_block_cached__sampling'

def setup_inputs():
    _rng = _Rng(jax.random.key(int.from_bytes(__import__("os").urandom(4), "little")))
    _w = (lambda a: (lambda t: t.astype(jnp.bfloat16) if jnp.issubdtype(t.dtype, jnp.floating) else t)(jnp.asarray(a)))
    B, Sq, D = 8, 4, 640
    Hq, Hkv, Sk, Dh = 32, 32, 4096, 192
    assert Hq % Hkv == 0, (Hq, Hkv)
    return {
        "x": _w((lambda *s: _rng.normal(s) * 0.8)(B, Sq, D)),
        "k_cache": _w((lambda *s: _rng.normal(s) * 0.8)(B, Hkv, Sk, Dh)),
        "v_cache": _w((lambda *s: _rng.normal(s) * 0.05)(B, Hkv, Sk, Dh)),
        "wq": _w((lambda *s: _rng.normal(s) * 0.8)(D, Hq * Dh) * (D ** -0.5)),
        "wo": _w((lambda *s: _rng.normal(s) * 0.05)(Hq * Dh, D) * ((Hq * Dh) ** -0.5)),
    }

def reference(x, k_cache, v_cache, wq, wo):
    B, Sq, D = x.shape
    Hq, Dh = 32, 192
    Hkv, Sk = k_cache.shape[1], k_cache.shape[2]
    W = min(4096, max(256, Sk // 4))
    rep = Hq // Hkv
    q = (lambda x, *d: x.transpose(*d))((x @ wq).reshape(B, Sq, Hq, Dh), 0, 2, 1, 3)
    k = jnp.repeat(k_cache[:, :, Sk - W:, :], rep, axis=1)
    v = jnp.repeat(v_cache[:, :, Sk - W:, :], rep, axis=1)
    scores = jnp.einsum("bhqd,bhkd->bhqk", q, k) * (Dh ** -0.5)
    p = _softmax(scores, axis=-1)
    o = jnp.einsum("bhqk,bhkd->bhqd", p, v)
    return (lambda x, *d: x.transpose(*d))(o, 0, 2, 1, 3).reshape(B, Sq, Hq * Dh) @ wo
```

```python
import functools
import jax
import jax.numpy as jnp
from jax import lax
from jax.experimental import pallas as pl
from jax.experimental.pallas import tpu as pltpu

HQ = 32
DH = 192
HP = 2
PW = HP * DH


def _kernel(x_hbm, k_hbm, v_hbm, wq_hbm, wo_hbm, o_ref,
            x_buf, x2_buf, q_buf, att_buf, acc_buf, k_buf, v_buf, wq_buf, wo_buf,
            sem_x, sem_k, sem_v, sem_wq, sem_wo, *, nk, nv, window, pk, pv):
    B, Sq, D = x_hbm.shape
    Sk = k_hbm.shape[3]
    n_pairs = HQ // HP
    n_steps = n_pairs * B
    R = HP * Sq
    scale = DH ** -0.5

    def k_copy(i):
        slot = i % nk
        return pltpu.make_async_copy(
            k_hbm.at[i % B, pl.ds((i // B) * HP, HP), :, pl.ds(Sk - window, window)],
            k_buf.at[slot], sem_k.at[slot])

    def v_copy(i):
        slot = i % nv
        return pltpu.make_async_copy(
            v_hbm.at[i % B, pl.ds((i // B) * HP, HP), :, pl.ds(Sk - window, window)],
            v_buf.at[slot], sem_v.at[slot])

    def wq_copy(p):
        return pltpu.make_async_copy(
            wq_hbm.at[:, pl.ds(pl.multiple_of(p * PW, 128), PW)], wq_buf, sem_wq.at[0])

    def wo_copy(p):
        return pltpu.make_async_copy(
            wo_hbm.at[pl.ds(pl.multiple_of(p * PW, 128), PW), :], wo_buf, sem_wo.at[0])

    x_copy = pltpu.make_async_copy(x_hbm, x_buf, sem_x.at[0])
    x_copy.start()
    wq_copy(0).start()
    for i in range(max(nk, nv)):
        if i < nk:
            k_copy(i).start(priority=pk)
        if i < nv:
            v_copy(i).start(priority=pv)
    wo_copy(0).start()

    x_copy.wait()
    for b in range(B):
        xb = x_buf[b].astype(jnp.float32)
        x2_buf[b * R:(b + 1) * R, :] = jnp.concatenate([xb] * HP, axis=0)
    acc_buf[...] = jnp.zeros_like(acc_buf)

    def own_head(rows):
        r = lax.broadcasted_iota(jnp.int32, (rows, PW), 0)
        c = lax.broadcasted_iota(jnp.int32, (rows, PW), 1)
        return ((r % R) // Sq) == (c // DH)

    def step(i, carry):
        p = i // B
        b = i % B

        @pl.when(b == 0)
        def _():
            wq_copy(p).wait()
            q = jnp.dot(x2_buf[...].astype(jnp.bfloat16), wq_buf[...],
                        preferred_element_type=jnp.float32)
            q_buf[...] = jnp.where(own_head(B * R), q, 0.0)

            @pl.when(p + 1 < n_pairs)
            def _():
                wq_copy(p + 1).start()

        row = pl.multiple_of(b * R, R)
        q2 = q_buf[pl.ds(row, R), :].astype(jnp.bfloat16)
        k_copy(i).wait()
        k2 = k_buf[i % nk].reshape(PW, window)
        s = jnp.dot(q2, k2, preferred_element_type=jnp.float32) * scale

        @pl.when(i + nk < n_steps)
        def _():
            k_copy(i + nk).start(priority=pk)

        m = jnp.max(s, axis=1, keepdims=True)
        e = jnp.exp(s - m)
        l = jnp.sum(e, axis=1, keepdims=True)
        v_copy(i).wait()
        v2 = v_buf[i % nv].reshape(PW, window)
        o = lax.dot_general(e.astype(jnp.bfloat16), v2, (((1,), (1,)), ((), ())),
                            preferred_element_type=jnp.float32)

        @pl.when(i + nv < n_steps)
        def _():
            v_copy(i + nv).start(priority=pv)

        att_buf[pl.ds(row, R), :] = jnp.where(own_head(R), o / l, 0.0)

        @pl.when(b == B - 1)
        def _():
            wo_copy(p).wait()
            acc_buf[...] += jnp.dot(att_buf[...].astype(jnp.bfloat16), wo_buf[...],
                                    preferred_element_type=jnp.float32)

            @pl.when(p + 1 < n_pairs)
            def _():
                wo_copy(p + 1).start()

        return carry

    lax.fori_loop(0, n_steps, step, 0)

    for b in range(B):
        r = acc_buf[b * R:(b + 1) * R, :]
        o_ref[b] = (r[:Sq] + r[Sq:]).astype(o_ref.dtype)


@jax.jit
def pallas_standalone__sliding_block_cached__sampling_kernel(
    x: jax.Array,
    k_cache: jax.Array,
    v_cache: jax.Array,
    wq: jax.Array,
    wo: jax.Array,
):
    nk, nv, pk, pv = 2, 2, 0, 1
    B, Sq, D = x.shape
    Sk = k_cache.shape[2]
    window = min(4096, max(256, Sk // 4))
    kt = jnp.swapaxes(k_cache, 2, 3)
    vt = jnp.swapaxes(v_cache, 2, 3)
    R = HP * Sq
    any_spec = pl.BlockSpec(memory_space=pl.ANY)
    return pl.pallas_call(
        functools.partial(_kernel, nk=nk, nv=nv, window=window, pk=pk, pv=pv),
        in_specs=[any_spec] * 5,
        out_specs=pl.BlockSpec(memory_space=pltpu.VMEM),
        out_shape=jax.ShapeDtypeStruct(x.shape, x.dtype),
        scratch_shapes=[
            pltpu.VMEM((B, Sq, D), x.dtype),
            pltpu.VMEM((B * R, D), jnp.float32),
            pltpu.VMEM((B * R, PW), jnp.float32),
            pltpu.VMEM((B * R, PW), jnp.float32),
            pltpu.VMEM((B * R, D), jnp.float32),
            pltpu.VMEM((nk, HP, DH, window), k_cache.dtype),
            pltpu.VMEM((nv, HP, DH, window), v_cache.dtype),
            pltpu.VMEM((D, PW), wq.dtype),
            pltpu.VMEM((PW, D), wo.dtype),
            pltpu.SemaphoreType.DMA((1,)),
            pltpu.SemaphoreType.DMA((nk,)),
            pltpu.SemaphoreType.DMA((nv,)),
            pltpu.SemaphoreType.DMA((1,)),
            pltpu.SemaphoreType.DMA((1,)),
        ],
        compiler_params=pltpu.CompilerParams(vmem_limit_bytes=64 * 1024 * 1024),
    )(x, kt, vt, wq, wo)
```

```python
import functools
import jax
import jax.numpy as jnp
from jax import lax
from jax.experimental import pallas as pl
from jax.experimental.pallas import tpu as pltpu

HQ = 32
DH = 192
HP = 2
PW = HP * DH


def kv_pieces(mode):
    out = []
    if mode == "whole0": return [(0, 384, 0, 1024, 0)]
    if mode == "whole1": return [(0, 384, 0, 1024, 1)]
    if mode == "kk3":
        for g in range(3):
            for c in range(8):
                for m in (g, g + 3):
                    out.append((m * 64, 64, c * 128, 128, c % 2))
    if mode == "seq":
        for g in range(6):
            for c in range(8):
                out.append((g * 64, 64, c * 128, 128, c % 2))
    return out


def _kernel(x_hbm, k_hbm, v_hbm, wq_hbm, wo_hbm, o_ref,
            x_buf, x2_buf, q_buf, att_buf, acc_buf, k_buf, v_buf, wq_buf, wo_buf,
            sem_x, sem_k, sem_v, sem_wq, sem_wo, *, nk, nv, window, kp, vp, compute):
    B, Sq, D = x_hbm.shape
    Sk = k_hbm.shape[2]
    n_pairs = HQ // HP
    n_steps = n_pairs * B
    R = HP * Sq
    scale = DH ** -0.5

    def start_window(src, buf, sem, n, pieces, i):
        slot = i % n
        row = (i // B) * PW
        for r0, nr, c0, nc, prio in pieces:
            pltpu.make_async_copy(
                src.at[i % B, pl.ds(pl.multiple_of(row + r0, 64), nr), pl.ds(Sk - window + c0, nc)],
                buf.at[slot, pl.ds(r0, nr), pl.ds(c0, nc)], sem.at[slot]).start(priority=prio)

    def wait_window(buf, sem, n, i):
        slot = i % n
        pltpu.make_async_copy(buf.at[slot], buf.at[slot], sem.at[slot]).wait()

    start_k = functools.partial(start_window, k_hbm, k_buf, sem_k, nk, kp)
    start_v = functools.partial(start_window, v_hbm, v_buf, sem_v, nv, vp)
    wait_k = functools.partial(wait_window, k_buf, sem_k, nk)
    wait_v = functools.partial(wait_window, v_buf, sem_v, nv)

    def wq_copy(p):
        return pltpu.make_async_copy(
            wq_hbm.at[:, pl.ds(pl.multiple_of(p * PW, 128), PW)], wq_buf, sem_wq.at[0])

    def wo_copy(p):
        return pltpu.make_async_copy(
            wo_hbm.at[pl.ds(pl.multiple_of(p * PW, 128), PW), :], wo_buf, sem_wo.at[0])

    x_copy = pltpu.make_async_copy(x_hbm, x_buf, sem_x.at[0])
    x_copy.start()
    wq_copy(0).start()
    for i in range(max(nk, nv)):
        if i < nk:
            start_k(i)
        if i < nv:
            start_v(i)
    wo_copy(0).start(priority=1)

    x_copy.wait()
    for b in range(B):
        xb = x_buf[b].astype(jnp.float32)
        x2_buf[b * R:(b + 1) * R, :] = jnp.concatenate([xb] * HP, axis=0)
    acc_buf[...] = jnp.zeros_like(acc_buf)

    def own_head(rows):
        r = lax.broadcasted_iota(jnp.int32, (rows, PW), 0)
        c = lax.broadcasted_iota(jnp.int32, (rows, PW), 1)
        return ((r % R) // Sq) == (c // DH)

    def step(i, carry):
        p = i // B
        b = i % B

        @pl.when(b == 0)
        def _():
            wq_copy(p).wait()
            if compute:
                q = jnp.dot(x2_buf[...].astype(jnp.bfloat16), wq_buf[...],
                            preferred_element_type=jnp.float32)
                q_buf[...] = jnp.where(own_head(B * R), q, 0.0)

            @pl.when(p + 1 < n_pairs)
            def _():
                wq_copy(p + 1).start()

        row = pl.multiple_of(b * R, R)
        if compute:
            q2 = q_buf[pl.ds(row, R), :].astype(jnp.bfloat16)
        wait_k(i)
        if compute:
            s = jnp.dot(q2, k_buf[i % nk], preferred_element_type=jnp.float32) * scale

        @pl.when(i + nk < n_steps)
        def _():
            start_k(i + nk)

        if compute:
            m = jnp.max(s, axis=1, keepdims=True)
            e = jnp.exp(s - m)
            l = jnp.sum(e, axis=1, keepdims=True)
        wait_v(i)
        if compute:
            o = lax.dot_general(e.astype(jnp.bfloat16), v_buf[i % nv], (((1,), (1,)), ((), ())),
                                preferred_element_type=jnp.float32)

        @pl.when(i + nv < n_steps)
        def _():
            start_v(i + nv)

        if compute:
            att_buf[pl.ds(row, R), :] = jnp.where(own_head(R), o / l, 0.0)

        @pl.when(b == B - 1)
        def _():
            wo_copy(p).wait()
            if compute:
                acc_buf[...] += jnp.dot(att_buf[...].astype(jnp.bfloat16), wo_buf[...],
                                        preferred_element_type=jnp.float32)

            @pl.when(p + 1 < n_pairs)
            def _():
                wo_copy(p + 1).start(priority=1)

        return carry

    lax.fori_loop(0, n_steps, step, 0)

    for b in range(B):
        r = acc_buf[b * R:(b + 1) * R, :]
        o_ref[b] = (r[:Sq] + r[Sq:]).astype(o_ref.dtype)


@jax.jit
def pallas_standalone__sliding_block_cached__sampling_kernel(x, k_cache, v_cache, wq, wo):
    if True:
        nk, nv, km, vm, nobc, compute = 2, 2, "kk3", "kk3", False, True
        B, Sq, D = x.shape
        Sk = k_cache.shape[2]
        window = min(4096, max(256, Sk // 4))
        kt = jnp.swapaxes(k_cache, 2, 3).reshape(B, HQ * DH, Sk)
        vt = jnp.swapaxes(v_cache, 2, 3).reshape(B, HQ * DH, Sk)
        R = HP * Sq
        any_spec = pl.BlockSpec(memory_space=pl.ANY)
        return pl.pallas_call(
            functools.partial(_kernel, nk=nk, nv=nv, window=window, kp=kv_pieces(km), vp=kv_pieces(vm), compute=compute),
            in_specs=[any_spec] * 5,
            out_specs=pl.BlockSpec(memory_space=pltpu.VMEM),
            out_shape=jax.ShapeDtypeStruct(x.shape, x.dtype),
            scratch_shapes=[
                pltpu.VMEM((B, Sq, D), x.dtype),
                pltpu.VMEM((B * R, D), jnp.float32),
                pltpu.VMEM((B * R, PW), jnp.float32),
                pltpu.VMEM((B * R, PW), jnp.float32),
                pltpu.VMEM((B * R, D), jnp.float32),
                pltpu.VMEM((nk, PW, window), k_cache.dtype),
                pltpu.VMEM((nv, PW, window), v_cache.dtype),
                pltpu.VMEM((D, PW), wq.dtype),
                pltpu.VMEM((PW, D), wo.dtype),
                pltpu.SemaphoreType.DMA((1,)),
                pltpu.SemaphoreType.DMA((nk,)),
                pltpu.SemaphoreType.DMA((nv,)),
                pltpu.SemaphoreType.DMA((1,)),
                pltpu.SemaphoreType.DMA((1,)),
            ],
            compiler_params=pltpu.CompilerParams(vmem_limit_bytes=64 * 1024 * 1024, disable_bounds_checks=nobc),
        )(x, kt, vt, wq, wo)
```

```python
import functools

import jax
import jax.numpy as jnp
from jax import lax
from jax.experimental import pallas as pl
from jax.experimental.pallas import tpu as pltpu

HQ = 32
DH = 192
PAIR = 2 * DH
LANES = 128
GROUP = 64
N_GROUPS = DH // GROUP
TAIL_ROWS = (384, 256, 128)
TAIL_PAIRS = sum(TAIL_ROWS) // PAIR
LEAD = 5


def _window_order(n_tiles):
    even, odd = (
        [(head, c) for c in range(parity, n_tiles, 2) for head in range(2)]
        for parity in range(2)
    )
    order = even[:LEAD]
    for j, piece in enumerate(odd):
        order += even[LEAD + j:LEAD + j + 1] + [piece]
    return order


def _kernel(x_hbm, kt_hbm, vt_hbm, wq_hbm, wo_hbm, out_ref,
            x_buf, xf_buf, q_buf, att_buf, acc_buf, k_buf, v_buf, wq_buf, wo_buf,
            x_sem, k_sem, v_sem, wq_sem, wo_sem, tail_sem):
    B, Sq, D = x_hbm.shape
    Sk = kt_hbm.shape[2]
    window = k_buf.shape[2]
    n_pairs = HQ // 2
    n_steps = n_pairs * B
    R = 2 * Sq
    scale = DH ** -0.5
    order = _window_order(window // LANES)

    def wait_filled(buf, sem):
        pltpu.make_async_copy(buf, buf, sem).wait()

    def start_window(src, buf, sem, i, also=None):
        slot = i % 2
        first_row = (i // B) * PAIR

        def group(g, carry):
            if also is not None:
                also(g)
            for head, c in order:
                row = pl.multiple_of(head * DH + g * GROUP, GROUP)
                pltpu.make_async_copy(
                    src.at[i % B,
                           pl.ds(pl.multiple_of(first_row + row, GROUP), GROUP),
                           pl.ds(Sk - window + c * LANES, LANES)],
                    buf.at[slot, pl.ds(row, GROUP), pl.ds(c * LANES, LANES)],
                    sem.at[slot],
                ).start(priority=c % 2)
            return carry

        lax.fori_loop(0, N_GROUPS, group, 0)

    def start_wq(p, row, rows, col, cols, priority):
        pltpu.make_async_copy(
            wq_hbm.at[pl.ds(row, rows), pl.ds(pl.multiple_of(p * PAIR + col, LANES), cols)],
            wq_buf.at[p % 2, pl.ds(row, rows), pl.ds(col, cols)],
            wq_sem.at[p % 2],
        ).start(priority=priority)

    def start_wo(p, row, rows, sem):
        pltpu.make_async_copy(
            wo_hbm.at[pl.ds(pl.multiple_of(p * PAIR + row, 16), rows), :],
            wo_buf.at[p % 2, pl.ds(row, rows), :],
            sem,
        ).start(priority=1)

    def project_q(p):
        wait_filled(wq_buf.at[p % 2], wq_sem.at[p % 2])
        q_buf[p % 2] = jnp.dot(xf_buf[...].astype(wq_buf.dtype), wq_buf[p % 2],
                               preferred_element_type=jnp.float32)

    tail = []
    for j, rows in enumerate(TAIL_ROWS):
        t, row = divmod(sum(TAIL_ROWS[:j]), PAIR)
        tail.append((n_pairs - TAIL_PAIRS + t, row, rows))

    x_copy = pltpu.make_async_copy(x_hbm, x_buf, x_sem.at[0])
    x_copy.start()
    for p in range(2):
        start_wq(p, 0, D, 0, PAIR, priority=p)
    for i in range(2):
        start_window(kt_hbm, k_buf, k_sem, i)
        start_window(vt_hbm, v_buf, v_sem, i)

    x_copy.wait()
    for b in range(B):
        xf_buf[b * Sq:(b + 1) * Sq, :] = x_buf[b].astype(jnp.float32)
    acc_buf[...] = jnp.zeros_like(acc_buf)
    att_buf[...] = jnp.zeros_like(att_buf)
    project_q(0)

    row_half = lax.broadcasted_iota(jnp.int32, (R, PAIR), 0) // Sq
    col_head = lax.broadcasted_iota(jnp.int32, (R, PAIR), 1) // DH

    def step(i, carry, stream_weights):
        p = i // B
        b = i % B

        @pl.when((b == B - 1) & (p + 1 < n_pairs))
        def _():
            project_q(p + 1)

        @pl.when((b == B // 2 - 1) & (p > 0) & (p <= n_pairs - TAIL_PAIRS))
        def _():
            prev = (p - 1) % 2
            wait_filled(wo_buf.at[prev], wo_sem.at[prev])
            acc_buf[...] += jnp.dot(att_buf[prev].astype(wo_buf.dtype), wo_buf[prev],
                                    preferred_element_type=jnp.float32)

        tile = pl.ds(pl.multiple_of((b // 2) * R, R), R)
        mine = row_half == b % 2
        q = q_buf[p % 2, tile, :]
        q = jnp.where(mine, q, pltpu.roll(q, Sq, 0))
        q = jnp.where(row_half == col_head, q, 0.0).astype(k_buf.dtype)

        wait_filled(k_buf.at[i % 2], k_sem.at[i % 2])
        s = jnp.dot(q, k_buf[i % 2], preferred_element_type=jnp.float32) * scale

        if stream_weights:
            start_window(
                kt_hbm, k_buf, k_sem, i + 2,
                lambda g: start_wq(p + 2, pl.multiple_of(b * (D // B), 16), D // B,
                                   pl.multiple_of(g * LANES, LANES), LANES, priority=0))
        else:
            @pl.when(i + 2 < n_steps)
            def _():
                start_window(kt_hbm, k_buf, k_sem, i + 2)

        e = jnp.exp(s - jnp.max(s, axis=1, keepdims=True))
        denom = jnp.sum(e, axis=1, keepdims=True)
        wait_filled(v_buf.at[i % 2], v_sem.at[i % 2])
        o = lax.dot_general(e.astype(v_buf.dtype), v_buf[i % 2], (((1,), (1,)), ((), ())),
                            preferred_element_type=jnp.float32)

        if stream_weights:
            rows = PAIR // (B * N_GROUPS)
            start_window(
                vt_hbm, v_buf, v_sem, i + 2,
                lambda g: start_wo(p, pl.multiple_of((b * N_GROUPS + g) * rows, 16), rows,
                                   wo_sem.at[p % 2]))
        else:
            @pl.when(i + 2 < n_steps)
            def _():
                start_window(vt_hbm, v_buf, v_sem, i + 2)

            @pl.when(i + 2 == n_steps - 1)
            def _():
                for j, (pair, row, rows) in enumerate(tail):
                    start_wo(pair, row, rows, tail_sem.at[j])

        o = o / denom
        o = jnp.where(row_half == col_head, o, pltpu.roll(o, Sq, 0))
        att_buf[p % 2, tile, :] = jnp.where(mine, o, att_buf[p % 2, tile, :])
        return carry

    n_streaming = (n_pairs - TAIL_PAIRS) * B
    lax.fori_loop(0, n_streaming, functools.partial(step, stream_weights=True), 0)
    lax.fori_loop(n_streaming, n_steps, functools.partial(step, stream_weights=False), 0)

    acc = acc_buf[...]
    for j, (pair, row, rows) in enumerate(tail):
        block = wo_buf.at[pair % 2, pl.ds(row, rows), :]
        wait_filled(block, tail_sem.at[j])
        acc += jnp.dot(att_buf[pair % 2, :, row:row + rows].astype(wo_buf.dtype), block[...],
                       preferred_element_type=jnp.float32)
    for b in range(B):
        out_ref[b] = acc[b * Sq:(b + 1) * Sq, :].astype(out_ref.dtype)


@jax.jit
def pallas_standalone__sliding_block_cached__sampling_kernel(
    x: jax.Array,
    k_cache: jax.Array,
    v_cache: jax.Array,
    wq: jax.Array,
    wo: jax.Array,
):
    B, Sq, D = x.shape
    Sk = k_cache.shape[2]
    window = min(4096, max(256, Sk // 4))
    assert k_cache.shape == v_cache.shape == (B, HQ, Sk, DH)
    assert wq.shape == (D, HQ * DH) and wo.shape == (HQ * DH, D)
    assert Sq == 4 and B % 2 == 0 and window % (2 * LANES) == 0 and Sk % LANES == 0
    assert D % (16 * B) == 0 and PAIR % (16 * B * N_GROUPS) == 0 and TAIL_PAIRS == 2

    kt = jnp.swapaxes(k_cache, 2, 3).reshape(B, HQ * DH, Sk)
    vt = jnp.swapaxes(v_cache, 2, 3).reshape(B, HQ * DH, Sk)
    return pl.pallas_call(
        _kernel,
        in_specs=[pl.BlockSpec(memory_space=pl.ANY)] * 5,
        out_specs=pl.BlockSpec(memory_space=pltpu.VMEM),
        out_shape=jax.ShapeDtypeStruct(x.shape, x.dtype),
        scratch_shapes=[
            pltpu.VMEM((B, Sq, D), x.dtype),
            pltpu.VMEM((B * Sq, D), jnp.float32),
            pltpu.VMEM((2, B * Sq, PAIR), jnp.float32),
            pltpu.VMEM((2, B * Sq, PAIR), jnp.float32),
            pltpu.VMEM((B * Sq, D), jnp.float32),
            pltpu.VMEM((2, PAIR, window), k_cache.dtype),
            pltpu.VMEM((2, PAIR, window), v_cache.dtype),
            pltpu.VMEM((2, D, PAIR), wq.dtype),
            pltpu.VMEM((2, PAIR, D), wo.dtype),
            pltpu.SemaphoreType.DMA((1,)),
            pltpu.SemaphoreType.DMA((2,)),
            pltpu.SemaphoreType.DMA((2,)),
            pltpu.SemaphoreType.DMA((2,)),
            pltpu.SemaphoreType.DMA((2,)),
            pltpu.SemaphoreType.DMA((len(TAIL_ROWS),)),
        ],
    )(x, kt, vt, wq, wo)
```
